```python
import jax
import jax.numpy as jnp

def _softmax(x, axis=-1):
    return jax.nn.softmax(x, axis=axis)
def _gelu(x):
    return jax.nn.gelu(x, approximate=True)
def _silu(x):
    return jax.nn.silu(x)
def _sigmoid(x):
    return jax.nn.sigmoid(x)
def _layernorm(x, axis=-1, eps=1e-5):
    m = jnp.mean(x, axis=axis, keepdims=True)
    v = jnp.var(x, axis=axis, keepdims=True)
    return (x - m) / jnp.sqrt(v + eps)
def _scatter_add(tgt, idx, src, axis=0):
    return tgt.at[idx].add(src)
def _segment_sum(src, seg, n):
    return jax.ops.segment_sum(src, seg, n)
class _Rng:
    def __init__(self, key):
        self._k = key
    def _next(self):
        self._k, sub = jax.random.split(self._k)
        return sub
    def normal(self, shape):
        return jax.random.normal(self._next(), shape, dtype=jnp.bfloat16)
    def randint(self, lo, hi, shape):
        return jax.random.randint(self._next(), shape, lo, hi, dtype=jnp.int32)
    def uniform(self, shape, lo=0.0, hi=1.0):
        return jax.random.uniform(self._next(), shape, jnp.bfloat16, lo, hi)
    def permutation(self, n):
        return jax.random.permutation(self._next(), n)


kernel_name = 'sequential_preLN__sliding_block__glu_gated_glu__prompt'

def _fwd_setup_inputs():
    _rng = _Rng(jax.random.key(int.from_bytes(__import__("os").urandom(4), "little")))
    _w = (lambda a: (lambda t: t.astype(jnp.bfloat16) if jnp.issubdtype(t.dtype, jnp.floating) else t)(jnp.asarray(a)))
    def _A_setup():
        B, S, D = 1, 2048, 512
        return {
            "x": _w((lambda *s: _rng.normal(s) * 0.05)(B, S, D)),
            "wqkv": _w((lambda *s: _rng.normal(s) * 0.05)(D, 3 * D)),
            "wo": _w((lambda *s: _rng.normal(s) * 0.05)(D, D)),
        }
    _A_in = _A_setup()

    def _B_setup():
        B, S, D, F = 1, 2048, 512, 1376
        return {
            "x": _w((lambda *s: _rng.normal(s) * 0.05)(B, S, D)),
            "w_gate": _w((lambda *s: _rng.normal(s) * 0.05)(D, F)),
            "w_up": _w((lambda *s: _rng.normal(s) * 0.05)(D, F)),
            "w_down": _w((lambda *s: _rng.normal(s) * 0.05)(F, D)),
        }
    _B_in = _B_setup()

    return {
        "A_x": _A_in["x"],
        "A_wqkv": _A_in["wqkv"],
        "A_wo": _A_in["wo"],
        "B_x": _B_in["x"],
        "B_w_gate": _B_in["w_gate"],
        "B_w_up": _B_in["w_up"],
        "B_w_down": _B_in["w_down"],
    }

def _fwd_reference(A_x, A_wqkv, A_wo, B_x, B_w_gate, B_w_up, B_w_down):
    def _A_ref(x, wqkv, wo):
        B, S, D = x.shape
        H = 32; Dh = D // H; W = 256
        qkv = (lambda x, *d: x.transpose(*d))((x @ wqkv).reshape(B, S, 3, H, Dh), 2, 0, 3, 1, 4)
        q, k, v = qkv[0], qkv[1], qkv[2]
        scores = jnp.einsum("bhqd,bhkd->bhqk", q, k) * (Dh ** -0.5)
        idx = jnp.arange(S)
        mask = (idx[:, None] - idx[None, :] >= 0) & (idx[:, None] - idx[None, :] < W)
        scores = jnp.where(mask[None, None], scores, -1e9)
        p = _softmax(scores, axis=-1)
        o = jnp.einsum("bhqk,bhkd->bhqd", p, v)
        return (lambda x, *d: x.transpose(*d))(o, 0, 2, 1, 3).reshape(B, S, D) @ wo

    def _B_ref(x, w_gate, w_up, w_down):
        g = jnp.einsum("bsd,df->bsf", x, w_gate)
        u = jnp.einsum("bsd,df->bsf", x, w_up)
        h = _sigmoid(g) * u
        return jnp.einsum("bsf,fd->bsd", h, w_down)

    x = A_x
    h = x + _A_ref(_layernorm(x, axis=-1), A_wqkv, A_wo)
    h2 = h + _B_ref(_layernorm(h, axis=-1), B_w_gate, B_w_up, B_w_down)
    return h2


def setup_inputs():
    _inp = _fwd_setup_inputs()
    _gk = jax.random.fold_in(jax.random.key(int.from_bytes(__import__("os").urandom(4), "little")), 2**31 - 1)
    _shapes = [[1, 2048, 512]]
    _dtypes = ['bfloat16']
    _gks = jax.random.split(_gk, len(_shapes))
    _gs = [jax.random.normal(k, s, dtype=jnp.dtype(d)) * 0.05 for k, s, d in zip(_gks, _shapes, _dtypes)]
    _inp["grad_out"] = _gs[0]
    return _inp

def reference(A_x, A_wqkv, A_wo, B_w_gate, B_w_up, B_w_down, B_x, grad_out):
    _const = dict(B_x=B_x)
    def _f(*_d):
        return _fwd_reference(**{'A_x': _d[0], 'A_wqkv': _d[1], 'A_wo': _d[2], 'B_w_gate': _d[3], 'B_w_up': _d[4], 'B_w_down': _d[5], **_const})
    _out, _vjp = jax.vjp(_f, A_x, A_wqkv, A_wo, B_w_gate, B_w_up, B_w_down)
    _grads = _vjp(grad_out)
    _out0 = jnp.asarray(_out)
    return (_out0, *[jnp.asarray(_g) for _g in _grads])
```

```python
import jax
import jax.numpy as jnp
import jax.experimental.pallas as pl
import jax.experimental.pallas.tpu as pltpu

S = 2048
D = 512
H = 32
DH = 16
W = 256
F = 1376
FP = 1408
QB = 128
KS = QB + W
R = 256
NSB = S // R
NQ = R // QB
NG = 4
RA = 512
XC = RA
NXC = S // XC
EPS = 1e-5
NEG = -1e9
WV = 2
SPLIT = 4
NSS = 2 * WV
LOG2E = 1.4426950408889634
LN2 = 0.6931471805599453

f32 = jnp.float32
bf16 = jnp.bfloat16


def _dot(a, b):
    return jnp.dot(a, b, preferred_element_type=f32)


def _dot_nt(a, b):
    return jax.lax.dot_general(a, b, (((1,), (1,)), ((), ())), preferred_element_type=f32)


def _dot_tn(a, b):
    return jax.lax.dot_general(a, b, (((0,), (0,)), ((), ())), preferred_element_type=f32)


def _ln_stats(x):
    m = jnp.mean(x, axis=-1, keepdims=True)
    xc = x - m
    v = jnp.mean(xc * xc, axis=-1, keepdims=True)
    r = jax.lax.rsqrt(v + EPS)
    return xc * r, r


def _ln_bwd(dy, y, r):
    return r * (dy - jnp.mean(dy, axis=-1, keepdims=True)
                - y * jnp.mean(dy * y, axis=-1, keepdims=True))


def _kernel(x_hbm, wqkv_hbm, wo_hbm, wg_hbm, wu_hbm, wd_hbm, go_hbm,
            out_hbm, dx_hbm, dwqkv_hbm, dwo_hbm, dwg_hbm, dwu_hbm, dwd_hbm,
            x_ref, wqkv_ref, wo_ref, go_ref, out_ref, dx_ref, dwqkv_ref, dwo_ref, dwgu_ref, dwd_ref,
            n1_s, kv_s, qkvT_s, oT_s, pT_s, wgu_s, wdp_s,
            n2_s, hh_s, dgu_s, dh_s, dhb_s, doT_s, dqkvT_s, s_scr, bias_s, rl_s, isem, osem):
    cp_xs = [pltpu.make_async_copy(x_hbm.at[pl.ds(i * XC, XC), :], x_ref.at[pl.ds(i * XC, XC), :], isem.at[7 + i])
             for i in range(NXC)]
    cp_wqkv = pltpu.make_async_copy(wqkv_hbm, wqkv_ref, isem.at[1])
    cp_wo = pltpu.make_async_copy(wo_hbm, wo_ref, isem.at[2])
    cp_wg = pltpu.make_async_copy(wg_hbm, wgu_s.at[0:F, :], isem.at[3])
    cp_wu = pltpu.make_async_copy(wu_hbm, wgu_s.at[FP:FP + F, :], isem.at[4])
    cp_wd = pltpu.make_async_copy(wd_hbm, wdp_s.at[0:F, :], isem.at[5])
    cp_go = pltpu.make_async_copy(go_hbm, go_ref, isem.at[6])
    cp_wqkv.start()
    for cp in cp_xs:
        cp.start()
    cp_wo.start()
    cp_wg.start()
    cp_wu.start()
    cp_wd.start()
    cp_go.start()
    kv_s[0:W, :] = jnp.zeros((W, 2 * D), bf16)
    qkvT_s[:, 0:W] = jnp.zeros((3 * D, W), bf16)
    wgu_s[F:FP, :] = jnp.zeros((FP - F, D), bf16)
    wgu_s[FP + F:2 * FP, :] = jnp.zeros((FP - F, D), bf16)
    wdp_s[F:FP, :] = jnp.zeros((FP - F, D), bf16)
    dqkvT_s[...] = jnp.zeros(dqkvT_s.shape, f32)
    cp_wqkv.wait()

    def phase_a(i, c):
        r0 = pl.multiple_of(i * RA, RA)
        pltpu.make_async_copy(x_hbm.at[pl.ds(r0, XC), :], x_ref.at[pl.ds(r0, XC), :], isem.at[7 + i]).wait()
        xb = x_ref[pl.ds(r0, RA), :].astype(f32)
        y, _ = _ln_stats(xb)
        n1 = y.astype(bf16)
        n1_s[pl.ds(r0, RA), :] = n1
        qkv = _dot(n1, wqkv_ref[...])
        kvb = qkv[:, D:].astype(bf16)
        kv_s[pl.ds(W + r0, RA), :] = kvb
        qb = (qkv[:, 0:D] * (DH ** -0.5 * LOG2E)).astype(bf16)
        qkvT_s[0:D, pl.ds(W + r0, RA)] = qb.T
        qkvT_s[D:, pl.ds(W + r0, RA)] = kvb.T
        return c
    with jax.named_scope('phA'):
        jax.lax.fori_loop(0, S // RA, phase_a, 0)

    cp_wo.wait()
    cp_wg.wait()
    cp_wu.wait()
    cp_wd.wait()
    cp_go.wait()
    hrow = jax.lax.broadcasted_iota(jnp.int32, (128, 8 * QB), 0) // DH
    hcol = jax.lax.broadcasted_iota(jnp.int32, (128, 8 * QB), 1) // QB
    hmask = hrow == hcol

    row1 = jax.lax.broadcasted_iota(jnp.int32, (KS, QB), 0)
    col1 = jax.lax.broadcasted_iota(jnp.int32, (KS, QB), 1)
    band1 = (col1 + W - row1 >= 0) & (col1 + W - row1 < W)

    def expand(t):
        return jnp.where(hmask, jnp.tile(t, (1, 8)), jnp.zeros((128, 8 * QB), t.dtype))

    def sweep(i, c):
        r0 = pl.multiple_of(i * R, R)

        def attn_fwd(ql, c2):
            q0 = pl.multiple_of(r0 + ql * QB, QB)
            valid = band1 & (row1 >= W - q0)
            bias_s[...] = jnp.where(valid, 0.0, NEG).astype(f32)
            hr = jax.lax.broadcasted_iota(jnp.int32, (128, QB), 0) // DH

            def s_mm(hh):
                g0 = (hh // 8) * 128
                qT = qkvT_s[g0:g0 + 128, pl.ds(W + q0, QB)]
                qm = jnp.where(hr == (hh % 8), qT, jnp.zeros_like(qT))
                for c in range(SPLIT):
                    cs = KS // SPLIT
                    kt = kv_s[pl.ds(q0 + c * cs, cs), g0:g0 + 128]
                    s_scr[hh % NSS, c * cs:(c + 1) * cs, :] = _dot(kt, qm)

            def softmax(hh):
                sm = [s_scr[hh % NSS, c * 64:(c + 1) * 64, :] + bias_s[c * 64:(c + 1) * 64, :] for c in range(6)]
                mx = [jnp.max(t, axis=0, keepdims=True) for t in sm]
                m = jnp.maximum(jnp.maximum(jnp.maximum(mx[0], mx[1]), jnp.maximum(mx[2], mx[3])),
                                jnp.maximum(mx[4], mx[5]))
                ls = []
                for c in range(6):
                    pc = jnp.exp2(sm[c] - m)
                    ls.append(jnp.sum(pc, axis=0, keepdims=True))
                    pT_s[ql * H + hh, c * 64:(c + 1) * 64, :] = pc.astype(bf16)
                l = (ls[0] + ls[1]) + (ls[2] + ls[3]) + (ls[4] + ls[5])
                rl_s[ql * H + hh] = 1.0 / l

            def pv(hh):
                hs = hh * DH
                vT = qkvT_s[2 * D + hs:2 * D + hs + DH, pl.ds(q0, KS)]
                oT = _dot(vT, pT_s[ql * H + hh]) * rl_s[ql * H + hh]
                oT_s[hs:hs + DH, pl.ds(q0, QB)] = oT.astype(bf16)

            for hh in range(WV):
                s_mm(hh)
            for w in range(H // WV):
                if w + 1 < H // WV:
                    for hh in range(WV):
                        s_mm((w + 1) * WV + hh)
                if w >= 1:
                    for hh in range(WV):
                        pv((w - 1) * WV + hh)
                for hh in range(WV):
                    softmax(w * WV + hh)
            for hh in range(WV):
                pv(H - WV + hh)
            return c2
        with jax.named_scope('attnF'):
            jax.lax.fori_loop(0, NQ, attn_fwd, 0)

        oT = oT_s[:, pl.ds(r0, R)]
        attn = _dot_tn(oT, wo_ref[...])
        hres = x_ref[pl.ds(r0, R), :].astype(f32) + attn
        y2, r2 = _ln_stats(hres)
        n2 = y2.astype(bf16)
        n2_s[pl.ds(r0, R), :] = n2
        gu = _dot_nt(n2, wgu_s[...])
        gg = gu[:, :FP]
        uu = gu[:, FP:]
        sg = jax.nn.sigmoid(gg)
        hh = (sg * uu).astype(bf16)
        hh_s[pl.ds(r0, R), :] = hh
        out_ref[pl.ds(r0, R), :] = (hres + _dot(hh, wdp_s[...])).astype(bf16)
        pltpu.make_async_copy(out_ref.at[pl.ds(r0, R), :], out_hbm.at[pl.ds(r0, R), :], osem.at[i]).start()
        go = go_ref[pl.ds(r0, R), :]
        dhh = _dot_nt(go, wdp_s[...])
        du = dhh * sg
        dg = du * uu * (1.0 - sg)
        dgu = jnp.concatenate([dg.astype(bf16), du.astype(bf16)], axis=1)
        dgu_s[pl.ds(r0, R), :] = dgu
        dn2 = _dot(dgu, wgu_s[...])
        dh = go.astype(f32) + _ln_bwd(dn2, y2, r2)
        dh_s[pl.ds(r0, R), :] = dh
        dhb = dh.astype(bf16)
        dhb_s[pl.ds(r0, R), :] = dhb
        doT_s[...] = _dot_nt(wo_ref[...], dhb).astype(bf16)

        def attn_bwd(ql, c2):
            q0 = pl.multiple_of(r0 + ql * QB, QB)
            ql0 = pl.multiple_of(ql * QB, QB)
            for g in range(NG):
                g0 = g * 128
                vt = kv_s[pl.ds(q0, KS), D + g0:D + g0 + 128]
                rl8 = jnp.concatenate([jnp.broadcast_to(rl_s[ql * H + g * 8 + h], (DH, QB)) for h in range(8)], axis=0)
                doT = doT_s[g0:g0 + 128, pl.ds(ql0, QB)].astype(f32)
                oT = oT_s[g0:g0 + 128, pl.ds(q0, QB)]
                prod = expand(doT * oT.astype(f32) * rl8)
                delta = jnp.sum(prod, axis=0, keepdims=True)
                doTs = (doT * rl8).astype(bf16)
                dpT = _dot(vt, expand(doTs))
                for h in range(8):
                    hs = g0 + h * DH
                    pn_h = pT_s[ql * H + g * 8 + h]
                    ds_h = (pn_h.astype(f32) * (dpT[:, h * QB:(h + 1) * QB] - delta[:, h * QB:(h + 1) * QB])).astype(bf16)
                    kT = qkvT_s[D + hs:D + hs + DH, pl.ds(q0, KS)]
                    qh = qkvT_s[hs:hs + DH, pl.ds(W + q0, QB)]
                    doh = doTs[h * DH:(h + 1) * DH]
                    dqkvT_s[hs:hs + DH, pl.ds(W + q0, QB)] = _dot(kT, ds_h) * (DH ** -0.5)
                    dqkvT_s[D + hs:D + hs + DH, pl.ds(q0, KS)] += _dot_nt(qh, ds_h) * LN2
                    dqkvT_s[2 * D + hs:2 * D + hs + DH, pl.ds(q0, KS)] += _dot_nt(doh, pn_h)
            return c2
        with jax.named_scope('attnB'):
            jax.lax.fori_loop(0, NQ, attn_bwd, 0)
        return c
    with jax.named_scope('sweep'):
        jax.lax.fori_loop(0, NSB, sweep, 0)

    def phase_f(i, c):
        r0 = pl.multiple_of(i * RA, RA)
        dqkvT = dqkvT_s[:, pl.ds(W + r0, RA)].astype(bf16)
        dn1 = _dot(wqkv_ref[...], dqkvT).T
        xb = x_ref[pl.ds(r0, RA), :].astype(f32)
        y1, r1 = _ln_stats(xb)
        dx_ref[pl.ds(r0, RA), :] = (dh_s[pl.ds(r0, RA), :] + _ln_bwd(dn1, y1, r1)).astype(bf16)
        pltpu.make_async_copy(dx_ref.at[pl.ds(r0, RA), :], dx_hbm.at[pl.ds(r0, RA), :], osem.at[NSB + i]).start()
        return c
    with jax.named_scope('phF'):
        jax.lax.fori_loop(0, S // RA, phase_f, 0)

    cpo = []

    def wg_qkv(j, c):
        c0 = pl.multiple_of(j * 256, 256)
        dq = dqkvT_s[pl.ds(c0, 256), W:].astype(bf16)
        dwqkv_ref[:, pl.ds(c0, 256)] = jax.lax.dot_general(
            n1_s[...], dq, (((0,), (1,)), ((), ())), preferred_element_type=f32).astype(bf16)
        return c
    jax.lax.fori_loop(0, 3 * D // 256, wg_qkv, 0)
    cpo.append(pltpu.make_async_copy(dwqkv_ref, dwqkv_hbm, osem.at[2 * NSB + 0]))
    cpo[-1].start()

    def wg_gu(j, c):
        c0 = pl.multiple_of(j * 128, 128)
        dwgu_ref[:, pl.ds(c0, 128)] = _dot_tn(dgu_s[...], n2_s[:, pl.ds(c0, 128)]).astype(bf16)
        return c
    jax.lax.fori_loop(0, D // 128, wg_gu, 0)
    cpo.append(pltpu.make_async_copy(dwgu_ref.at[0:F, :], dwg_hbm, osem.at[2 * NSB + 2]))
    cpo[-1].start()
    cpo.append(pltpu.make_async_copy(dwgu_ref.at[FP:FP + F, :], dwu_hbm, osem.at[2 * NSB + 3]))
    cpo[-1].start()

    def wg_d(j, c):
        c0 = pl.multiple_of(j * 128, 128)
        dwd_ref[:, pl.ds(c0, 128)] = _dot_tn(hh_s[...], go_ref[:, pl.ds(c0, 128)]).astype(bf16)
        return c
    jax.lax.fori_loop(0, D // 128, wg_d, 0)
    cpo.append(pltpu.make_async_copy(dwd_ref.at[0:F, :], dwd_hbm, osem.at[2 * NSB + 4]))
    cpo[-1].start()
    dwo_ref[...] = _dot(oT_s[...], dhb_s[...]).astype(bf16)
    cpo.append(pltpu.make_async_copy(dwo_ref, dwo_hbm, osem.at[2 * NSB + 1]))
    cpo[-1].start()
    for i in range(NSB):
        pltpu.make_async_copy(out_ref.at[pl.ds(i * R, R), :], out_hbm.at[pl.ds(i * R, R), :], osem.at[i]).wait()
    for i in range(S // RA):
        pltpu.make_async_copy(dx_ref.at[pl.ds(i * RA, RA), :], dx_hbm.at[pl.ds(i * RA, RA), :], osem.at[NSB + i]).wait()
    for cp in cpo:
        cp.wait()


@jax.jit
def pallas_sequential_preLN__sliding_block__glu_gated_glu__prompt_kernel(
    A_x: jax.Array,
    A_wqkv: jax.Array,
    A_wo: jax.Array,
    B_x: jax.Array,
    B_w_gate: jax.Array,
    B_w_up: jax.Array,
    B_w_down: jax.Array,
    grad_out: jax.Array,
):
    x = A_x.reshape(S, D)
    go = grad_out.reshape(S, D)
    out_shape = (
        jax.ShapeDtypeStruct((S, D), bf16),
        jax.ShapeDtypeStruct((S, D), bf16),
        jax.ShapeDtypeStruct((D, 3 * D), bf16),
        jax.ShapeDtypeStruct((D, D), bf16),
        jax.ShapeDtypeStruct((F, D), bf16),
        jax.ShapeDtypeStruct((F, D), bf16),
        jax.ShapeDtypeStruct((F, D), bf16),
    )
    scratch = [
        pltpu.VMEM((S, D), bf16),
        pltpu.VMEM((D, 3 * D), bf16),
        pltpu.VMEM((D, D), bf16),
        pltpu.VMEM((S, D), bf16),
        pltpu.VMEM((S, D), bf16),
        pltpu.VMEM((S, D), bf16),
        pltpu.VMEM((D, 3 * D), bf16),
        pltpu.VMEM((D, D), bf16),
        pltpu.VMEM((2 * FP, D), bf16),
        pltpu.VMEM((FP, D), bf16),
        pltpu.VMEM((S, D), bf16),
        pltpu.VMEM((S + W, 2 * D), bf16),
        pltpu.VMEM((3 * D, S + W), bf16),
        pltpu.VMEM((D, S), bf16),
        pltpu.VMEM((NQ * H, KS, QB), bf16),
        pltpu.VMEM((2 * FP, D), bf16),
        pltpu.VMEM((FP, D), bf16),
        pltpu.VMEM((S, D), bf16),
        pltpu.VMEM((S, FP), bf16),
        pltpu.VMEM((S, 2 * FP), bf16),
        pltpu.VMEM((S, D), f32),
        pltpu.VMEM((S, D), bf16),
        pltpu.VMEM((D, R), bf16),
        pltpu.VMEM((3 * D, S + W), f32),
        pltpu.VMEM((NSS, KS, QB), f32),
        pltpu.VMEM((KS, QB), f32),
        pltpu.VMEM((NQ * H, 1, QB), f32),
        pltpu.SemaphoreType.DMA((7 + NXC,)),
        pltpu.SemaphoreType.DMA((2 * NSB + 5,)),
    ]
    outs = pl.pallas_call(
        _kernel,
        out_shape=out_shape,
        in_specs=[pl.BlockSpec(memory_space=pl.ANY)] * 7,
        out_specs=[pl.BlockSpec(memory_space=pl.ANY)] * 7,
        scratch_shapes=scratch,
        compiler_params=pltpu.CompilerParams(vmem_limit_bytes=120 * 1024 * 1024),
    )(x, A_wqkv, A_wo, B_w_gate.T, B_w_up.T, B_w_down, go)
    out, dx, dwqkv, dwo, dwgT, dwuT, dwd = outs
    return (out.reshape(1, S, D), dx.reshape(1, S, D), dwqkv, dwo, dwgT.T, dwuT.T, dwd)
```
